```python
import os as _os
_os.environ.setdefault('JAX_PLATFORMS', 'cpu')
import jax
import jax.numpy as jnp

def _softmax(x, axis=-1):
    return jax.nn.softmax(x, axis=axis)

def _gelu(x):
    return jax.nn.gelu(x, approximate=True)

def _silu(x):
    return jax.nn.silu(x)

def _sigmoid(x):
    return jax.nn.sigmoid(x)

def _layernorm(x, axis=-1, eps=1e-05):
    m = jnp.mean(x, axis=axis, keepdims=True)
    v = jnp.var(x, axis=axis, keepdims=True)
    return (x - m) / jnp.sqrt(v + eps)

def _scatter_add(tgt, idx, src, axis=0):
    return tgt.at[idx].add(src)

def _segment_sum(src, seg, n):
    return jax.ops.segment_sum(src, seg, n)

class _Rng:

    def __init__(self, key):
        self._k = key

    def _next(self):
        self._k, sub = jax.random.split(self._k)
        return sub

    def normal(self, shape):
        return jax.random.normal(self._next(), shape, dtype=jnp.bfloat16)

    def randint(self, lo, hi, shape):
        return jax.random.randint(self._next(), shape, lo, hi, dtype=jnp.int32)

    def uniform(self, shape, lo=0.0, hi=1.0):
        return jax.random.uniform(self._next(), shape, jnp.bfloat16, lo, hi)

    def permutation(self, n):
        return jax.random.permutation(self._next(), n)
kernel_name = 'adaLN_cond__linear_attn_block__swiglu_ffn__prompt'

def setup_inputs():
    _rng = _Rng(jax.random.key(int.from_bytes(__import__("os").urandom(4), "little")))
    _w = lambda a: (lambda t: t.astype(jnp.bfloat16) if jnp.issubdtype(t.dtype, jnp.floating) else t)(jnp.asarray(a))

    def _A_setup():
        B, S, D = (1, 2048, 640)
        return {'x': _w((lambda *s: _rng.normal(s) * 0.05)(B, S, D)), 'wqkv': _w((lambda *s: _rng.normal(s) * 0.8)(D, 3 * D)), 'wo': _w((lambda *s: _rng.normal(s) * 0.05)(D, D))}
    _A_in = _A_setup()

    def _B_setup():
        B, S, D, F = (1, 2048, 640, 1728)
        return {'x': _w((lambda *s: _rng.normal(s) * 0.05)(B, S, D)), 'w_gate': _w((lambda *s: _rng.normal(s) * 0.05)(D, F)), 'w_up': _w((lambda *s: _rng.normal(s) * 0.05)(D, F)), 'w_down': _w((lambda *s: _rng.normal(s) * 0.05)(F, D))}
    _B_in = _B_setup()
    return {'A_x': _A_in['x'], 'A_wqkv': _A_in['wqkv'], 'A_wo': _A_in['wo'], 'B_x': _B_in['x'], 'B_w_gate': _B_in['w_gate'], 'B_w_up': _B_in['w_up'], 'B_w_down': _B_in['w_down'], 'c': _w((lambda *s: _rng.normal(s) * 0.05)(1, 640) * 8.0), 'w_mod': _w((lambda *s: _rng.normal(s) * 0.05)(640, 6 * 640) * 640 ** (-0.5) * 8.0)}

def reference(A_x, A_wqkv, A_wo, B_x, B_w_gate, B_w_up, B_w_down, c, w_mod):

    def _A_ref(x, wqkv, wo):
        B, S, D = x.shape
        H = 32
        Dh = D // H
        qkv = (lambda x, *d: x.transpose(*d))((x @ wqkv).reshape(B, S, 3, H, Dh), 2, 0, 3, 1, 4)
        q, k, v = (qkv[0], qkv[1], qkv[2])
        phi = lambda t: jnp.where(t > 0, t + 1, jnp.exp(t)) + 1e-06
        pq, pk = (phi(q), phi(k))
        kv = jnp.einsum('bhsd,bhse->bhde', pk, v)
        z = jnp.einsum('bhsd->bhd', pk)
        num = jnp.einsum('bhqd,bhde->bhqe', pq, kv)
        den = jnp.einsum('bhqd,bhd->bhq', pq, z)[..., None] + 1e-06
        o = num / den
        return (lambda x, *d: x.transpose(*d))(o, 0, 2, 1, 3).reshape(B, S, D) @ wo

    def _B_ref(x, w_gate, w_up, w_down):
        g = _silu(x @ w_gate)
        u = x @ w_up
        return g * u @ w_down
    x = A_x
    mod = (_silu(c) @ w_mod).reshape(c.shape[0], 6, 1, -1)
    sa, ca, ga, sb, cb, gb = (mod[:, 0].copy(), mod[:, 1].copy(), mod[:, 2].copy(), mod[:, 3].copy(), mod[:, 4].copy(), mod[:, 5].copy())
    h = _layernorm(x, axis=-1) * (1 + ca) + sa
    x = x + ga * _A_ref(h, A_wqkv, A_wo)
    h = _layernorm(x, axis=-1) * (1 + cb) + sb
    x = x + gb * _B_ref(h, B_w_gate, B_w_up, B_w_down)
    return x
```

```python
import jax
import jax.experimental.pallas as pl
import jax.experimental.pallas.tpu as pltpu
import jax.numpy as jnp
import numpy as np
from jax import lax

S, D, F, H = 2048, 640, 1728, 32
DH = D // H
L = 128
ND = D // L
FL = F // L * L
NF = FL // L + 1
T = 512
TH = T // 2
bf16, f32 = jnp.bfloat16, jnp.float32


def _scheme(m, k, n, rows, order=None):
    rows = [rows[r] for r in order] if order else rows
    val = {"+": 1, "0": 0, "-": -1}
    u, v, w = (np.array([[val[ch] for ch in row.split()[d]] for row in rows]) for d in range(3))
    for r in range(len(rows)):
        if not (u[r] > 0).any():
            u[r], w[r] = -u[r], -w[r]
        if not (v[r] > 0).any():
            v[r], w[r] = -v[r], -w[r]
    want = np.zeros((m * k, k * n, m * n), int)
    for i in range(m):
        for j in range(k):
            for l in range(n):
                want[i * k + j, j * n + l, i * n + l] = 1
    assert (np.einsum("ra,rb,rc->abc", u, v, w) == want).all()
    return k, n, u, v, w


_STRASSEN = _scheme(2, 2, 2, (
    "+00+ +00+ +00+", "00++ +000 00+-", "+000 0+0- 0+0+", "000+ -0+0 +0+0",
    "++00 000+ -+00", "-0+0 ++00 000+", "0+0- 00++ +000",
))
_HOPCROFT_KERR = (
    "00+0-00+0- 00000000000000-0000000000 0000000-0-",
    "000000000+ 0000+0000-000000000+0-+0- 0000+0000-",
    "0+0+000000 000+0000-0000000000000000 0-0-000000",
    "-00000+000 0+000-0000000000000000000 0-000-0000",
    "00000+0+00 00-0000000000000000000000 +0+00-0-00",
    "--00+00000 000000000000000000000-000 --00+++00-",
    "0++000+000 0000000+000-0000000000000 0-0000++00",
    "000000+000 0-0000+-0000000+-00000000 0-0000+000",
    "000+0--0+0 000-00000000000+000000000 ++0-0000+0",
    "0++000++00 00000000000+0000000000000 000000++00",
    "000-000--0 0000000000000-000-0000000 00+-0000+0",
    "000-00+000 000-0000+000000+-00000000 0+000000+0",
    "00-0+00000 0000000000000000000000+00 00+0+00-0-",
    "00000+000+ 0000-0000+000000000000000 00000-000-",
    "0000000--0 00000000000000000+0000000 00+-000-+0",
    "0000000+00 00+00000000+-0+00+0000000 0000000-00",
    "00+0-0000- 00000000000000+0000000+00 0000+00-0-",
    "+0000+0000 +-00-0000+-00000000000000 00000+0000",
    "-0-00-0-00 0000000000-00000000000000 +0+0000000",
    "0--0000000 0000000-00000000000000000 0++000--00",
    "-0000-0-00 00-0000000+00000000000000 +0+00-0000",
    "+00000000- 0000-0000+0000000000+-000 0000--0000",
    "00000--0+0 000000000000000+000000000 --0+0++0-0",
    "++00-0000- 000000000-00000000000+000 0000---00+",
    "00-0000000 0000000+00+0--00000000-00 00+0000000",
    "++0-0++0-0 000+000000000000000000000 --0+000000",
    "00++000++0 0000000000000+00000000000 00-+000000",
    "+000+00000 00000000000000000000-+000 -000-00000",
    "000+0000+0 000-000000000+0-+0-+00000 00000000-0",
    "00000000-- 0000000000000000000+00000 00000000--",
    "-000000000 -0+00+00000000000000+-000 +0000-0000",
    "++00000000 000+0+000000000000000+000 ++00000000",
    "000--00000 00000000000000000000000+0 000--00000",
    "0-0000-000 000+0-+0-00-0000000000000 0-00000000",
    "000+00000- 0000000000000000000-000+0 0000-000-0",
    "0000+0000+ 000000000+0000+00000-+0-+ 0000+00000",
    "000-000000 000-0000+000000-0--0000+0 000+0000-0",
    "000000-0-0 000000000000000-+00000000 000000-0-0",
    "00000++000 0+0000000+00000+000000000 00000++000",
    "++00-++00- 000000000-000000000000000 00000++00-",
)
GU_ORDER = (23, 33, 5, 22, 21, 39, 13, 1, 35, 34, 32, 27, 31, 25, 8, 28, 36, 14, 26, 10,
            9, 2, 6, 19, 15, 11, 3, 7, 37, 17, 38, 30, 18, 20, 4, 24, 0, 12, 29, 16)
DN_ORDER = (6, 31, 13, 18, 33, 19, 36, 0, 14, 15, 7, 28, 8, 11, 25, 26, 29, 38, 3, 9,
            17, 4, 32, 24, 2, 16, 27, 12, 23, 10, 34, 1, 35, 5, 37, 21, 39, 20, 30, 22)
GU_WAVE = 4
Q_FIRST = 2
TIE_STEP = 9
G_ORDER = (0, 6, 5, 4, 3, 2, 1)
Q_ORDER = (4, 0, 2, 5, 3, 1, 6)
A_ORDER = (2, 4, 3, 6, 1, 5, 0)
D_ORDER = (6, 2, 0, 3, 4, 5, 1)

_POOL = dict(h=ND * S, m=ND * D, wq=ND * D, hc=7 * S, mc=28 * L, wqc=28 * L, wgu=(2 * NF - 1) // ND * 40 * L,
             wd=(40 + 14) * 2 * L, ha=40 * TH, h2=ND * T, aa=(40 + 7) * 2 * TH)
_AT = {k: sum(list(_POOL.values())[:i]) for i, k in enumerate(_POOL)}


def _dot(a, b):
    return jnp.dot(a, b, preferred_element_type=f32)


def _dot_nt(a, b):
    return lax.dot_general(a, b, (((1,), (1,)), ((), ())), preferred_element_type=f32)


def _phi(t):
    return jnp.where(t > 0, t + 1.0, jnp.exp(t)) + 1e-6


def _layernorm(x):
    xc = x - jnp.mean(x, axis=-1, keepdims=True)
    return xc * lax.rsqrt(jnp.mean(xc * xc, axis=-1, keepdims=True) + 1e-5)


def _swiglu(half_g, u):
    return (half_g * jnp.tanh(half_g) + half_g) * u


def _tile(j, n=1):
    return slice(j * L, (j + n) * L)


def _single(coefs):
    nz = np.flatnonzero(coefs)
    return int(nz[0]) if len(nz) == 1 and coefs[nz[0]] > 0 else None


def _signed_sum(coefs, get):
    pos = [i for i, c in enumerate(coefs) if c > 0]
    neg = [i for i, c in enumerate(coefs) if c < 0]
    if pos:
        acc = get(pos[0])
        for i in pos[1:]:
            acc = acc + get(i)
    else:
        acc, neg = -get(neg[0]), neg[1:]
    for i in neg:
        acc = acc - get(i)
    return acc


def _signed_sums(rows, vals, share=True):
    rows, vals = [{i: int(c) for i, c in enumerate(r) if c} for r in rows], list(vals)
    while share:
        count = {}
        for r in rows:
            for i in r:
                for j in r:
                    if i < j:
                        count[i, j, r[i] * r[j]] = count.get((i, j, r[i] * r[j]), 0) + 1
        if not count or max(count.values()) < 2:
            break
        i, j, sign = max(sorted(count), key=count.get)
        vals.append(vals[i] + vals[j] if sign > 0 else vals[i] - vals[j])
        for r in rows:
            if i in r and j in r and r[i] * r[j] == sign:
                r[len(vals) - 1] = r.pop(i)
                del r[j]
    return [_signed_sum([r.get(i, 0) for i in range(len(vals))], vals.__getitem__) for r in rows]


def _accumulate(acc, w, prods):
    for o in range(len(acc)):
        co = [wr[o] for wr in w]
        if not any(co):
            continue
        if acc[o] is None:
            acc[o] = _signed_sum(co, prods.__getitem__)
        elif any(c > 0 for c in co):
            acc[o] = acc[o] + _signed_sum(co, prods.__getitem__)
        else:
            acc[o] = acc[o] - _signed_sum([-c for c in co], prods.__getitem__)


def _kernel(c_hbm, x_hbm, wqkv_hbm, wo_hbm, wg_hbm, wu_hbm, wd_hbm, wmod_hbm, o_hbm,
            c_v, x_v, wqkv_v, wo_v, wg_v, wu_v, wd_v, wmod_v, wkT_v, tmp_v,
            g_v, gq_v, wf_v, z_v, k0_v, x1_v, a_v, o_v, pool_v, sems, osems):
    su, sv, sw = _STRASSEN[2:]
    _, _, gu_u, gu_v, gu_w = _scheme(2, ND, ND, _HOPCROFT_KERR, GU_ORDER)
    dn_plan = ((_scheme(2, ND, ND, _HOPCROFT_KERR, DN_ORDER), 0, 0, 0), (_STRASSEN, 2 * ND, 80, 80))
    fh = D // 2

    def get(row, n):
        return pool_v[pl.ds(row, n), :]

    def put(row, val):
        pool_v[pl.ds(row, val.shape[0]), :] = val.astype(bf16)

    def get_wide(base, rows, r, n, tiles):
        return jnp.concatenate([get(base + j * rows + r, n) for j in range(tiles)], axis=1)

    def put_wide(base, rows, r, val):
        for j in range(val.shape[1] // L):
            put(base + j * rows + r, val[:, _tile(j)])

    copies = dict(
        c=(c_hbm, c_v),
        x1=(x_hbm.at[T:2 * T], x_v.at[T:2 * T]), x2=(x_hbm.at[2 * T:S], x_v.at[2 * T:S]),
        wq=(wqkv_hbm.at[:, 0:D], wqkv_v.at[:, 0:D]),
        wv=(wqkv_hbm.at[:, 2 * D:3 * D], wqkv_v.at[:, 2 * D:3 * D]),
        mb=(wmod_hbm.at[:, 2 * D:6 * D], wmod_v.at[:, 2 * D:6 * D]),
        wo=(wo_hbm, wo_v), wg=(wg_hbm, wg_v.at[0:F]), wu=(wu_hbm, wu_v),
        wx=(wu_hbm.at[FL:F], wg_v.at[F:FL + L]),
        wd=(wd_hbm, wd_v.at[0:F]),
    )
    for r in range(0, T, TH):
        copies["xa%d" % r] = (x_hbm.at[r:r + TH], x_v.at[r:r + TH])
    for j in range(ND):
        copies["wk%d" % j] = (wqkv_hbm.at[_tile(j), D:2 * D], wqkv_v.at[_tile(j), D:2 * D])
        copies["sa%d" % j] = (wmod_hbm.at[:, _tile(j)], wmod_v.at[:, _tile(j)])
        copies["ca%d" % j] = (wmod_hbm.at[:, _tile(ND + j)], wmod_v.at[:, _tile(ND + j)])
    dma = {k: pltpu.make_async_copy(s, d, sems.at[i]) for i, (k, (s, d)) in enumerate(copies.items())}

    def start(*names):
        for k in names:
            dma[k].start()

    def wait(*names):
        for k in names:
            dma[k].wait()

    events = [("c",)]
    for j in range(ND):
        if j * TH < T:
            events.append(("xa%d" % (j * TH),))
        events.append(("wk%d" % j, "ca%d" % j, "sa%d" % j))
    ahead = 4
    for names in events[:ahead]:
        start(*names)
    ca1, sa, normed, done = [], [], [], []
    for e, names in enumerate(events):
        wait(*names)
        if e + ahead < len(events):
            start(*events[e + ahead])
        if e == len(events) - 2:
            start("x1")
        had = [(j, r) for j in range(len(ca1)) for r in normed]
        if names == ("c",):
            cc = c_v[...].astype(f32)
            c_is_nan = jnp.broadcast_to(cc[:, 0:L] != cc[:, 0:L], (8, L))
            sc8 = jnp.broadcast_to(cc * jax.nn.sigmoid(cc), (8, D)).astype(bf16)
        elif len(names) == 1:
            r = len(normed) * TH
            x1_v[r:r + TH, :] = _layernorm(x_v[r:r + TH, :].astype(f32))
            normed.append(r)
        else:
            j = len(ca1)
            wkT_v[:, _tile(j)] = wqkv_v[_tile(j), D:2 * D].T
            ca1.append(1.0 + _dot(sc8, wmod_v[:, _tile(ND + j)])[0:1])
            sa.append(_dot(sc8, wmod_v[:, _tile(j)])[0:1])
        have = [(j, r) for j in range(len(ca1)) for r in normed]
        for j, r in have:
            if (j, r) not in had:
                hj = x1_v[r:r + TH, _tile(j)] * ca1[j] + sa[j]
                put(_AT["h"] + j * S + r, hj)
                x1_v[r:r + TH, _tile(j)] = hj
        ready = [q for q in (have if e == len(events) - 1 else had) if q not in done]
        for r in normed:
            js = [j for j, q in ready if q == r]
            if js:
                kj = _dot_nt(wkT_v[:, _tile(js[0], len(js))], get_wide(_AT["h"] + js[0] * S, S, r, TH, len(js)))
                if js[0] == 0:
                    k0_v[:, r:r + TH] = kj
                else:
                    k0_v[:, r:r + TH] += kj
        done += ready
    ca1, sa = jnp.concatenate(ca1, axis=1), jnp.concatenate(sa, axis=1)

    def h_sums(r0, r, halves):
        for p in range(7):
            if _single(su[p]) is None:
                put_wide(_AT["hc"] + r0 * 7 + p * T, TH, r,
                         _signed_sum(su[p], lambda t: halves[t // 2][:, _tile(2 * (t % 2), 2)]))

    def h_sum(r0, p):
        t = _single(su[p])
        if t is not None:
            return get_wide(_AT["h"] + 2 * (t % 2) * S, S, r0 + t // 2 * TH, TH, 2)
        return get_wide(_AT["hc"] + r0 * 7 + p * T, TH, 0, TH, 2)

    def norm1(r0):
        for r in range(0, TH, 16):
            halves = [_layernorm(x_v[o:o + 16, :].astype(f32)) * ca1 + sa for o in (r0 + r, r0 + TH + r)]
            for i in range(2):
                put_wide(_AT["h"], S, r0 + i * TH + r, halves[i])
            h_sums(r0, r, halves)

    def phi_k(r):
        if r == 0:
            return [_phi(k0_v[l * fh:(l + 1) * fh, i * TH:(i + 1) * TH]) for i in range(2) for l in range(2)]
        y = [_dot_nt(wkT_v[...], get_wide(_AT["h"], S, r + i * TH, TH, ND)) for i in range(2)]
        return [_phi(y[i][l * fh:(l + 1) * fh]) for i in range(2) for l in range(2)]

    def gram(r, p):
        def add(ref, idx, val):
            if r == 0:
                ref[idx] = val
            else:
                ref[idx] += val
        for l in range(2):
            add(z_v, (slice(l * fh, (l + 1) * fh), slice(None)),
                _signed_sum([1] * (T // L), lambda t: p[t * L // TH * 2 + l][:, _tile(t % (TH // L))]))
        pb = jnp.concatenate([jnp.concatenate([p[l], p[2 + l]], axis=1) for l in range(2)], axis=0).astype(bf16)
        for q in G_ORDER:
            add(gq_v, q, _dot(_signed_sum(sw[q], p.__getitem__).astype(bf16), h_sum(r, q)))
        add(g_v, (slice(None), _tile(4)), _dot(pb, get(_AT["h"] + 4 * S + r, T)))

    for r in range(0, TH, 16):
        h_sums(0, r, [x1_v[o:o + 16, 0:4 * L] for o in (r, TH + r)])
    wd_v[F:FL + L, :] = jnp.zeros((FL + L - F, D), bf16)
    pk = phi_k(0)
    wait("x1")
    start("x2", "wq", "wv", "wo")
    norm1(T)
    gram(0, pk)
    wait("x2")
    start("mb")
    for r in range(2 * T, S, T):
        norm1(r)
    for r in range(T, S, T):
        if r == 2 * T:
            wait("wq", "wv", "wo")
            start("wg", "wu", "wx", "wd")
        gram(r, phi_k(r))
    for t in range(4):
        g_v[t % 2 * fh:(t % 2 + 1) * fh, _tile(2 * (t // 2), 2)] = _signed_sum(sv[:, t], lambda q: gq_v[q])

    for j in range(ND):
        tmp_v[j] = wqkv_v[_tile(j), 0:D].astype(f32).T
    for d in range(DH):
        w = [tmp_v[j, pl.ds(d, H, stride=DH), :] for j in range(ND)]
        for j in range(ND):
            put(_AT["wq"] + j * D + d * H, w[j])
            wf_v[d * H:(d + 1) * H, _tile(j)] = w[j]
    for p in range(7):
        put_wide(_AT["wqc"] + p * 4 * L, 2 * L, 0,
                 _signed_sum(sv[p], lambda t: wf_v[_tile(2 * (t % 2), 2), _tile(2 * (t // 2), 2)]))

    z_v[...] = jnp.broadcast_to(jnp.sum(z_v[...], axis=1, keepdims=True), (D, L))
    z_row = jnp.concatenate([z_v[pl.ds(d, H, stride=DH), :] for d in range(DH)], axis=0).T[0:1, :]

    side, side_vals = [], []

    def after_side_work(lhs):
        if side:
            side.pop(0)()
        bits = [pltpu.bitcast(w[0:16].astype(bf16), jnp.int32) for w in side_vals[TIE_STEP - 1::TIE_STEP]]
        side_vals.clear()
        lhs = lhs()
        if not bits:
            return lhs
        t = bits[0]
        for b in bits[1:]:
            t = t | b
        head = pltpu.bitcast(jnp.where(c_is_nan, t, pltpu.bitcast(lhs[0:16, 0:L], jnp.int32)), bf16)
        return jnp.concatenate([jnp.concatenate([head, lhs[0:16, L:]], axis=1), lhs[16:]], axis=0)

    def project(order, dot, lhs_sum, rhs_sums, lhs, rhs_last_k, rhs_last_n):
        acc = [None] * 4
        for p in order:
            _accumulate(acc, [sw[p]], [dot(after_side_work(lambda: lhs_sum(p)),
                                           get_wide(rhs_sums + p * 4 * L, 2 * L, 0, 2 * L, 2))])
        y, y4 = dot(lhs[:, _tile(4)], rhs_last_k), dot(lhs, rhs_last_n)
        return [jnp.concatenate([acc[2 * i + l] + y[i * TH:(i + 1) * TH, _tile(2 * l, 2)] for l in range(2)]
                                + [y4[i * TH:(i + 1) * TH]], axis=1) for i in range(2)]

    def query(r):
        out = []
        for q in project(Q_ORDER, _dot_nt, lambda p: h_sum(r, p), _AT["wqc"], get_wide(_AT["h"], S, r, T, ND),
                         get(_AT["wq"] + 4 * D, 4 * L), get_wide(_AT["wq"], D, 4 * L, L, ND)):
            pq = _phi(q)
            t = pq * z_row
            s = t[:, 0:L]
            for j in range(1, ND):
                s = s + t[:, _tile(j)]
            s = s + pltpu.roll(s, 2 * H, 1)
            s = s + pltpu.roll(s, H, 1)
            rcp = 1.0 / (s + 1e-6)
            out.append(jnp.concatenate([pq[:, _tile(j)] * rcp for j in range(ND)], axis=1))
        return out

    def attend(r, pq):
        y = project(A_ORDER, _dot,
                    lambda p: _signed_sum(su[p], lambda t: pq[t // 2][:, _tile(2 * (t % 2), 2)]).astype(bf16),
                    _AT["mc"], jnp.concatenate(pq, axis=0).astype(bf16),
                    get_wide(_AT["m"], D, 4 * L, L, 4), get(_AT["m"] + 4 * D, D))
        for i in range(2):
            rows = slice(r + i * TH, r + (i + 1) * TH)
            x1_v[rows, :] = x_v[rows, :].astype(f32) + ga * y[i]

    pqs = [query(i * T) for i in range(Q_FIRST)]

    spans = [(j * L // DH * DH // 16 * 16, pl.cdiv(pl.cdiv((j + 1) * L, DH) * DH, 16) * 16) for j in range(ND)]
    kvs = []
    for j, (lo, hi) in enumerate(spans):
        kv = _dot(g_v[lo:hi, :].astype(bf16), wqkv_v[:, _tile(2 * ND + j)])
        k_head = (lax.broadcasted_iota(jnp.int32, kv.shape, 0) + lo) // DH
        v_head = (lax.broadcasted_iota(jnp.int32, kv.shape, 1) + j * L) // DH
        kvs.append(jnp.where(k_head == v_head, kv, 0.0).astype(bf16))
    for j, (lo, hi) in enumerate(spans):
        mj = _dot(kvs[j], wo_v[_tile(j), :])
        old = spans[j - 1][1] if j else lo
        for l in range(ND):
            if old > lo:
                tmp_v[l, lo:old, :] += mj[0:old - lo, _tile(l)]
            tmp_v[l, old:hi, :] = mj[old - lo:, _tile(l)]
    for l in range(ND):
        for d in range(DH):
            w = tmp_v[l, pl.ds(d, H, stride=DH), :]
            put(_AT["m"] + l * D + d * H, w)
            wf_v[d * H:(d + 1) * H, _tile(l)] = w
    for p in range(7):
        put_wide(_AT["mc"] + p * 4 * L, 2 * L, 0,
                 _signed_sum(sv[p], lambda t: wf_v[_tile(2 * (t // 2), 2), _tile(2 * (t % 2), 2)]))

    wait("mb", "wg", "wu", "wx", "wd")

    def modulation(v):
        return _dot(sc8, wmod_v[:, v * D:(v + 1) * D])[0:1]

    n_gu = 2 * NF - 1
    groups = n_gu // ND

    def gu_tile(t, j, r=0, n=L):
        return (wu_v if t % 2 else wg_v)[t // 2 * L + r:t // 2 * L + r + n, _tile(j)]

    def weight_sums(coefs, blocks, row):
        keep = [r for r in range(len(coefs)) if _single(coefs[r]) is None]
        for r, w in zip(keep, _signed_sums(coefs[keep], [b.astype(f32) for b in blocks])):
            put(row(r), w)
            side_vals.append(w)

    def gu_sums(g, r0):
        weight_sums(gu_v, [gu_tile(g * ND + t % ND, t // ND, r0, 16) for t in range(ND * ND)],
                    lambda r: _AT["wgu"] + (g * 40 + r) * L + r0)

    def dn_sums(plan, q, r0):
        (k, n, _, v, _), k0, w0, _ = plan
        for g in range(ND // n):
            weight_sums(v, [wd_v[pl.ds((k0 + q * k + t // n) * L + r0, 16), _tile(g * n + t % n)] for t in range(k * n)],
                        lambda r: _AT["wd"] + (w0 + (g * len(v) + r) * 2 + q) * L + r0)

    def norm2(r0, r):
        h2 = [_layernorm(x1_v[pl.ds(r0 + i * TH + r, 16), :]) * cb1 + sb for i in range(2)]
        for p, w in enumerate(_signed_sums(gu_u, [h2[t // ND][:, _tile(t % ND)] for t in range(2 * ND)])):
            put(_AT["ha"] + p * TH + r, w)
            side_vals.append(w)
        for i in range(2):
            put_wide(_AT["h2"], T, i * TH + r, h2[i])

    ga = modulation(2)
    side += [lambda g=g, r=r: gu_sums(g, r) for g in range(groups) for r in range(0, L, 16)]
    side += [lambda p=p, q=q, r=r: dn_sums(p, q, r) for p in dn_plan for q in range(2) for r in range(0, L, 16)]
    for i in range(S // T):
        if len(pqs) < min(i + Q_FIRST, S // T):
            pqs.append(query(len(pqs) * T))
        attend(i * T, pqs[i])
    sb = modulation(3)
    cb1, sb = 0.5 + 0.5 * modulation(4), 0.5 * sb
    for r in range(0, TH, 16):
        norm2(0, r)
    for fn in side:
        fn()
    gb = 2.0 * modulation(5)

    def out_copy(i):
        rows = pl.ds(i * T if isinstance(i, int) else pl.multiple_of(i * T, T), T)
        return pltpu.make_async_copy(o_v.at[rows], o_hbm.at[rows], osems.at[i])

    def ffn(i, carry):
        r0 = pl.multiple_of(i * T, T)
        tiles = {}

        def activate():
            for t in sorted(set(t for t, _ in tiles)):
                for b in range(2):
                    rows = slice(b * TH, (b + 1) * TH)
                    if t == n_gu - 1:
                        gu = tiles.pop((t, b))
                        lane = lax.broadcasted_iota(jnp.int32, gu.shape, 1)
                        a_v[rows, _tile(t // 2)] = jnp.where(lane < F - FL, _swiglu(gu, pltpu.roll(gu, F - FL, 1)), 0.0)
                    elif t % 2 == 0 and (t + 1, b) in tiles:
                        a_v[rows, _tile(t // 2)] = _swiglu(tiles.pop((t, b)), tiles.pop((t + 1, b)))

        def gu_sum(g, r):
            t = _single(gu_v[r])
            return get(_AT["wgu"] + (g * 40 + r) * L, L) if t is None else gu_tile(g * ND + t % ND, t // ND)

        def act_sums(plan, q, r):
            (k, _, u, _, _), k0, _, s0 = plan
            blocks = [a_v[t // k * TH + r:t // k * TH + r + 16, _tile(k0 + q * k + t % k)] for t in range(2 * k)]
            for p, w in enumerate(_signed_sums(u, blocks, share=False)):
                if _single(u[p]) is None:
                    put(_AT["aa"] + (s0 + p * 2 + q) * TH + r, w)

        def act_sum(plan, p):
            (k, _, u, _, _), k0, _, s0 = plan
            t = _single(u[p])
            if t is None:
                return get_wide(_AT["aa"] + (s0 + p * 2) * TH, TH, 0, TH, 2)
            return jnp.concatenate([a_v[t // k * TH:(t // k + 1) * TH, _tile(k0 + q * k + t % k)]
                                    for q in range(2)], axis=1).astype(bf16)

        def dn_sum(plan, g, p, q):
            (k, n, _, v, _), k0, w0, _ = plan
            t = _single(v[p])
            if t is None:
                return get(_AT["wd"] + (w0 + (g * len(v) + p) * 2 + q) * L, L)
            return wd_v[_tile(k0 + q * k + t // n), _tile(g * n + t % n)]

        for t in range(groups * ND, n_gu):
            y = _dot_nt(get_wide(_AT["h2"], T, 0, T, ND), jnp.concatenate([gu_tile(t, j) for j in range(ND)], axis=1))
            for b in range(2):
                tiles[t, b] = y[b * TH:(b + 1) * TH]
        activate()
        pending = [(p[1] + (q + 1) * p[0][0] - 1, p, q) for p in dn_plan for q in range(2)]
        for g in range(groups):
            now = [(p, q, r) for t, p, q in pending if t < g * ND // 2 for r in range(0, TH, 16)]
            pending = [x for x in pending if x[0] >= g * ND // 2]
            acc, waves = [None] * (2 * ND), range(0, 40, GU_WAVE)
            for n, p0 in enumerate(waves):
                for x in now[n * len(now) // len(waves):(n + 1) * len(now) // len(waves)]:
                    act_sums(*x)
                ps = range(p0, min(p0 + GU_WAVE, 40))
                _accumulate(acc, [gu_w[p] for p in ps], [_dot_nt(get(_AT["ha"] + p * TH, TH), gu_sum(g, p)) for p in ps])
            for b in range(2):
                for l in range(ND):
                    tiles[g * ND + l, b] = acc[b * ND + l]
            activate()
        for _, p, q in pending:
            for r in range(0, TH, 16):
                act_sums(p, q, r)

        res = [x1_v[pl.ds(r0 + b * TH, TH), _tile(l)] for b in range(2) for l in range(ND)]
        nxt = pl.multiple_of(jnp.minimum(i + 1, S // T - 1) * T, T)
        for r in range(0, TH, 16):
            norm2(nxt, r)
        acc = [None] * (2 * ND)
        y = _dot(a_v[:, _tile(2 * ND, 4)].astype(bf16), wd_v[_tile(2 * ND, 4), _tile(4)])
        acc[4], acc[ND + 4] = y[0:TH], y[TH:T]
        for plan in dn_plan:
            _, n, u, _, w = plan[0]
            for g in range(ND // n):
                for p in D_ORDER if len(u) == 7 else range(len(u)):
                    co = [w[p][b * n + l - g * n] if g * n <= l < (g + 1) * n else 0 for b in range(2) for l in range(ND)]
                    _accumulate(acc, [co], [_dot(act_sum(plan, p),
                                                 jnp.concatenate([dn_sum(plan, g, p, q) for q in range(2)], axis=0))])
        for b in range(2):
            for l in range(ND):
                o_v[pl.ds(r0 + b * TH, TH), _tile(l)] = (res[b * ND + l] + gb[:, _tile(l)] * acc[b * ND + l]).astype(bf16)
        out_copy(i).start()
        return carry

    lax.fori_loop(0, S // T, ffn, None)
    for i in range(S // T):
        out_copy(i).wait()


@jax.jit
def pallas_adaLN_cond__linear_attn_block__swiglu_ffn__prompt_kernel(
    A_x: jax.Array,
    A_wqkv: jax.Array,
    A_wo: jax.Array,
    B_x: jax.Array,
    B_w_gate: jax.Array,
    B_w_up: jax.Array,
    B_w_down: jax.Array,
    c: jax.Array,
    w_mod: jax.Array,
):
    del B_x
    hbm = pl.BlockSpec(memory_space=pltpu.HBM)
    vmem = pltpu.VMEM
    out = pl.pallas_call(
        _kernel,
        out_shape=jax.ShapeDtypeStruct((S, D), bf16),
        in_specs=[hbm] * 8,
        out_specs=hbm,
        scratch_shapes=[
            vmem((1, D), bf16), vmem((S, D), bf16), vmem((D, 3 * D), bf16), vmem((D, D), bf16),
            vmem((FL + L, D), bf16), vmem((F, D), bf16), vmem((FL + L, D), bf16), vmem((D, 6 * D), bf16),
            vmem((D, D), bf16), vmem((ND, D, L), f32),
            vmem((D, D), f32), vmem((7, D // 2, 2 * L), f32), vmem((D, D), f32), vmem((D, L), f32),
            vmem((D, T), f32), vmem((S, D), f32), vmem((T, FL + L), f32), vmem((S, D), bf16),
            vmem((sum(_POOL.values()), L), bf16),
            pltpu.SemaphoreType.DMA((13 + 3 * ND,)), pltpu.SemaphoreType.DMA((S // T,)),
        ],
        compiler_params=pltpu.CompilerParams(
            vmem_limit_bytes=110 * 1024 * 1024,
            flags={"XLA_TPU_EVENLY_DISTRIBUTE_CRITICAL_NODES": True},
        ),
    )(c, A_x.reshape(S, D), A_wqkv, A_wo, B_w_gate.T, B_w_up.T, B_w_down, w_mod)
    return out.reshape(1, S, D)
```
